```python
import os as _os
_os.environ.setdefault("JAX_PLATFORMS", "cpu")
import jax
import jax.numpy as jnp

def _softmax(x, axis=-1):
    return jax.nn.softmax(x, axis=axis)
def _gelu(x):
    return jax.nn.gelu(x, approximate=True)
def _silu(x):
    return jax.nn.silu(x)
def _sigmoid(x):
    return jax.nn.sigmoid(x)
def _layernorm(x, axis=-1, eps=1e-5):
    m = jnp.mean(x, axis=axis, keepdims=True)
    v = jnp.var(x, axis=axis, keepdims=True)
    return (x - m) / jnp.sqrt(v + eps)
def _scatter_add(tgt, idx, src, axis=0):
    return tgt.at[idx].add(src)
def _segment_sum(src, seg, n):
    return jax.ops.segment_sum(src, seg, n)
class _Rng:
    def __init__(self, key):
        self._k = key
    def _next(self):
        self._k, sub = jax.random.split(self._k)
        return sub
    def normal(self, shape):
        return jax.random.normal(self._next(), shape, dtype=jnp.bfloat16)
    def randint(self, lo, hi, shape):
        return jax.random.randint(self._next(), shape, lo, hi, dtype=jnp.int32)
    def uniform(self, shape, lo=0.0, hi=1.0):
        return jax.random.uniform(self._next(), shape, jnp.bfloat16, lo, hi)
    def permutation(self, n):
        return jax.random.permutation(self._next(), n)


kernel_name = 'parallel_sum__mha_block__swiglu_ffn__prompt'

def setup_inputs():
    _rng = _Rng(jax.random.key(int.from_bytes(__import__("os").urandom(4), "little")))
    _w = (lambda a: (lambda t: t.astype(jnp.bfloat16) if jnp.issubdtype(t.dtype, jnp.floating) else t)(jnp.asarray(a)))
    def _A_setup():
        B, S, D, H = 1, 2048, 640, 32
        return {
            "x": _w((lambda *s: _rng.normal(s) * 0.05)(B, S, D)),
            "wqkv": _w((lambda *s: _rng.normal(s) * 0.1)(D, 3 * D)),
            "wo": _w((lambda *s: _rng.normal(s) * 0.05)(D, D)),
        }
    _A_in = _A_setup()

    def _B_setup():
        B, S, D, F = 1, 2048, 640, 1536
        return {
            "x": _w((lambda *s: _rng.normal(s) * 0.05)(B, S, D)),
            "w_gate": _w((lambda *s: _rng.normal(s) * 0.05)(D, F)),
            "w_up": _w((lambda *s: _rng.normal(s) * 0.05)(D, F)),
            "w_down": _w((lambda *s: _rng.normal(s) * 0.05)(F, D)),
        }
    _B_in = _B_setup()

    return {
        "A_x": _A_in["x"],
        "A_wqkv": _A_in["wqkv"],
        "A_wo": _A_in["wo"],
        "B_x": _B_in["x"],
        "B_w_gate": _B_in["w_gate"],
        "B_w_up": _B_in["w_up"],
        "B_w_down": _B_in["w_down"],
    }

def reference(A_x, A_wqkv, A_wo, B_x, B_w_gate, B_w_up, B_w_down):
    def _A_ref(x, wqkv, wo):
        B, S, D = x.shape
        H = 32
        Dh = D // H
        qkv = (lambda x, *d: x.transpose(*d))((x @ wqkv).reshape(B, S, 3, H, Dh), 2, 0, 3, 1, 4)
        q, k, v = qkv[0], qkv[1], qkv[2]
        scores = jnp.einsum("bhqd,bhkd->bhqk", q, k) * (Dh ** -0.5)
        p = _softmax(scores, axis=-1)
        o = jnp.einsum("bhqk,bhkd->bhqd", p, v)
        return (lambda x, *d: x.transpose(*d))(o, 0, 2, 1, 3).reshape(B, S, D) @ wo

    def _B_ref(x, w_gate, w_up, w_down):
        g = _silu(x @ w_gate)
        u = x @ w_up
        return (g * u) @ w_down

    x = A_x
    xn = _layernorm(x, axis=-1)
    return x + _A_ref(xn, A_wqkv, A_wo) + _B_ref(xn, B_w_gate, B_w_up, B_w_down)
```

```python
import functools
import math

import jax
import jax.numpy as jnp
from jax import lax
import jax.experimental.pallas as pl
import jax.experimental.pallas.tpu as pltpu

S = 2048
D = 640
H = 32
DH = 20
F = 1536
R = 24
TQ = 512
KC = 128
LAG = 2
NQ = S // TQ
NC = S // KC
NU = H * NQ
RB = 512
NRB = S // RB
EPS = 1e-5
QSCALE = (DH ** -0.5) * math.log2(math.e)

STRADDLE = ((6, 112, 8), (12, 208, 32), (19, 320, 60), (25, 416, 84))

f32 = jnp.float32
bf16 = jnp.bfloat16


def _head_geom(h):
    c0 = h * DH
    j = c0 // 128
    start = j * 128
    r = c0 - start
    for (hs, st, rr) in STRADDLE:
        is_h = h == hs
        j = jnp.where(is_h, 5, j)
        start = jnp.where(is_h, st, start)
        r = jnp.where(is_h, rr, r)
    return j, start, r


def _kernel(x_hbm, wqkv_hbm, wo_hbm, wg_hbm, wu_hbm, wd_hbm, out_hbm,
            x_v, wqkv_v, wo_v, wg_v, wu_v, wd_v,
            wqvt_v, wkx_v, xn_v, k_v, qt_v, vt_v, ot_v, sa, sb, ma, mb, mpart, out_v,
            sem_x, sem_w, sem_o):
    def x_copy(b):
        return pltpu.make_async_copy(x_hbm.at[pl.ds(b * RB, RB)], x_v.at[pl.ds(b * RB, RB)], sem_x.at[b])

    w_copies = [pltpu.make_async_copy(src, dst, sem_w.at[i]) for i, (src, dst) in enumerate(
        ((wqkv_hbm, wqkv_v), (wg_hbm, wg_v), (wu_hbm, wu_v), (wd_hbm, wd_v), (wo_hbm, wo_v)))]

    def out_copy(b):
        return pltpu.make_async_copy(out_v.at[pl.ds(b * RB, RB)], out_hbm.at[pl.ds(b * RB, RB)], sem_o.at[b])

    x_copy(0).start()
    w_copies[0].start()
    for b in range(1, NRB):
        x_copy(b).start()
    for c in w_copies[1:]:
        c.start()

    w_copies[0].wait()
    wqvt_v[0:D, :] = wqkv_v[:, 0:D].T
    wqvt_v[D:2 * D, :] = wqkv_v[:, 2 * D:3 * D].T
    src = lax.broadcasted_iota(jnp.int32, (D, 128), 0)
    dst = lax.broadcasted_iota(jnp.int32, (D, 128), 1)
    perm = jnp.zeros((D, 128), jnp.bool_)
    for (hs, st, rr) in STRADDLE:
        perm = perm | ((dst >= rr) & (dst < rr + DH) & (src == dst + (hs * DH - rr)))
    perm = jnp.where(perm, 1.0, 0.0).astype(bf16)
    wkx_v[...] = jnp.dot(wqkv_v[:, D:2 * D], perm, preferred_element_type=f32).astype(bf16)

    for b in range(NRB):
        rows = pl.ds(b * RB, RB)
        x_copy(b).wait()
        x = x_v[rows, :].astype(f32)
        mu = jnp.mean(x, axis=-1, keepdims=True)
        xc = x - mu
        var = jnp.mean(xc * xc, axis=-1, keepdims=True)
        xn = (xc * lax.rsqrt(var + EPS)).astype(bf16)
        xn_v[rows, :] = xn
        kk = jnp.dot(xn, wqkv_v[:, D:2 * D], preferred_element_type=f32).astype(bf16)
        for j in range(5):
            k_v[j, rows, :] = kk[:, j * 128:(j + 1) * 128]
        k_v[5, rows, :] = jnp.dot(xn, wkx_v[...], preferred_element_type=f32).astype(bf16)
        qt = lax.dot_general(wqvt_v[0:D, :], xn, (((1,), (1,)), ((), ())), preferred_element_type=f32)
        qt_v[:, rows] = (qt * QSCALE).astype(bf16)
        vt = lax.dot_general(wqvt_v[D:2 * D, :], xn, (((1,), (1,)), ((), ())), preferred_element_type=f32)
        tail = jnp.where(lax.broadcasted_iota(jnp.int32, (R - DH, RB), 0) == 0, 1.0, 0.0).astype(f32)
        for h in range(H):
            vt_v[h, 0:DH, rows] = vt[h * DH:(h + 1) * DH, :]
            vt_v[h, DH:R, rows] = tail

    sbuf = (sa, sb)
    mbuf = (ma, mb)

    def getw(i):
        i = jnp.minimum(i, NU - 1)
        h = i // NQ
        qb = i % NQ
        j, start, r = _head_geom(h)
        q0 = pl.multiple_of(qb * TQ, TQ)
        w = qt_v[pl.ds(pl.multiple_of(start, 16), 128), pl.ds(q0, TQ)]
        rws = lax.broadcasted_iota(jnp.int32, (128, TQ), 0)
        w = jnp.where((rws >= r) & (rws < r + DH), w, jnp.zeros_like(w))
        return j, w

    def qk_chunk(jw, c, s_ref, m):
        j, w = jw
        s = jnp.dot(k_v[j, pl.ds(c * KC, KC), :], w, preferred_element_type=f32)
        s_ref[pl.ds(c * KC, KC), :] = s
        mc = jnp.max(s.reshape(KC // 8, 8, TQ), axis=0)
        return mc if m is None else jnp.maximum(m, mc)

    def pv_chunk(h, c, s_ref, m, o):
        p = jnp.exp2(s_ref[pl.ds(c * KC, KC), :] - m).astype(bf16)
        oc = jnp.dot(vt_v[h, :, pl.ds(c * KC, KC)], p, preferred_element_type=f32)
        return oc if o is None else o + oc

    def fin(mn, m_ref):
        m_ref[...] = jnp.broadcast_to(jnp.max(mn, axis=0, keepdims=True), (8, TQ))

    jw = getw(0)
    mn = None
    for c in range(NC):
        mn = qk_chunk(jw, c, sa, mn)
    fin(mn, ma)
    jw = getw(1)
    mn = None
    for c in range(LAG):
        mn = qk_chunk(jw, c, sb, mn)
    mpart[...] = mn

    def head_body(h, carry):
        i0 = NQ * h
        mn = mpart[...]
        jw1 = getw(i0 + 1)
        for u in range(NQ):
            m = mbuf[u % 2][0:1, :]
            jw2 = getw(i0 + u + 2)
            o = None
            mn2 = None
            for c in range(NC):
                if c + LAG < NC:
                    mn = qk_chunk(jw1, c + LAG, sbuf[(u + 1) % 2], mn)
                    if c + LAG == NC - 1:
                        fin(mn, mbuf[(u + 1) % 2])
                    o = pv_chunk(h, c, sbuf[u % 2], m, o)
                else:
                    o = pv_chunk(h, c, sbuf[u % 2], m, o)
                    mn2 = qk_chunk(jw2, c + LAG - NC, sbuf[u % 2], mn2)
            ot_v[h, :, u * TQ:(u + 1) * TQ] = o * (1.0 / o[DH:DH + 1, :])
            mn = mn2
            jw1 = jw2
        mpart[...] = mn
        return carry

    lax.fori_loop(0, H, head_body, 0)

    for c in w_copies[1:]:
        c.wait()
    for b in range(NRB):
        rows = pl.ds(b * RB, RB)
        xn = xn_v[rows, :]
        g = jnp.dot(xn, wg_v[...], preferred_element_type=f32)
        u = jnp.dot(xn, wu_v[...], preferred_element_type=f32)
        hmid = (g * jax.nn.sigmoid(g) * u).astype(bf16)
        ffn = jnp.dot(hmid, wd_v[...], preferred_element_type=f32)
        ot = jnp.concatenate([ot_v[h, 0:DH, rows] for h in range(H)], axis=0).astype(bf16)
        attn = lax.dot_general(ot, wo_v[...], (((0,), (0,)), ((), ())), preferred_element_type=f32)
        out_v[rows, :] = (x_v[rows, :].astype(f32) + attn + ffn).astype(bf16)
        out_copy(b).start()
    for b in range(NRB):
        out_copy(b).wait()


@jax.jit
def pallas_parallel_sum__mha_block__swiglu_ffn__prompt_kernel(
    A_x: jax.Array,
    A_wqkv: jax.Array,
    A_wo: jax.Array,
    B_x: jax.Array,
    B_w_gate: jax.Array,
    B_w_up: jax.Array,
    B_w_down: jax.Array,
):
    x = A_x.reshape(S, D)
    any_spec = pl.BlockSpec(memory_space=pl.ANY)
    out = pl.pallas_call(
        _kernel,
        out_shape=jax.ShapeDtypeStruct((S, D), bf16),
        in_specs=[any_spec] * 6,
        out_specs=any_spec,
        scratch_shapes=[
            pltpu.VMEM((S, D), bf16),
            pltpu.VMEM((D, 3 * D), bf16),
            pltpu.VMEM((D, D), bf16),
            pltpu.VMEM((D, F), bf16),
            pltpu.VMEM((D, F), bf16),
            pltpu.VMEM((F, D), bf16),
            pltpu.VMEM((2 * D, D), bf16),
            pltpu.VMEM((D, 128), bf16),
            pltpu.VMEM((S, D), bf16),
            pltpu.VMEM((6, S, 128), bf16),
            pltpu.VMEM((D, S), bf16),
            pltpu.VMEM((H, R, S), f32),
            pltpu.VMEM((H, R, S), f32),
            pltpu.VMEM((S, TQ), f32),
            pltpu.VMEM((S, TQ), f32),
            pltpu.VMEM((8, TQ), f32),
            pltpu.VMEM((8, TQ), f32),
            pltpu.VMEM((8, TQ), f32),
            pltpu.VMEM((S, D), bf16),
            pltpu.SemaphoreType.DMA((NRB,)),
            pltpu.SemaphoreType.DMA((5,)),
            pltpu.SemaphoreType.DMA((NRB,)),
        ],
        compiler_params=pltpu.CompilerParams(vmem_limit_bytes=100 * 2**20),
    )(x, A_wqkv, A_wo, B_w_gate, B_w_up, B_w_down)
    return out.reshape(1, S, D)
```

```python
import math

import jax
import jax.numpy as jnp
from jax import lax
import jax.experimental.pallas as pl
import jax.experimental.pallas.tpu as pltpu

S = 2048
D = 640
H = 32
DH = 20
NP = H // 2
F = 1536
R = 24
TQ = 256
KC = 128
LAG = 2
NQ = S // TQ
NC = S // KC
RB = 512
NRB = S // RB
SB = 256
FR = S // NP
EPS = 1e-5
QSCALE = (DH ** -0.5) * math.log2(math.e)

KR = 64
G = 2.0 ** -6
C = 1.5 * 2.0 ** 23 * G
RLIM = 160.0
MARGIN = 1.03
ONES2 = 0x3F803F80

f32 = jnp.float32
bf16 = jnp.bfloat16
u32 = jnp.uint32


def _kernel(x_hbm, wqkv_hbm, wo_hbm, wg_hbm, wu_hbm, wd_hbm, out_hbm,
            x_v, wq_v, wk_v, wv_v, wo_v, wg_v, wu_v, wd_v,
            wqvt_v, xn_v, kn_v, kp_v, qm_v, ie_v, vt_v, ot_v,
            s1a, s1b, s2a, s2b, m1a, m1b, m2a, m2b, mp1, mp2,
            kmax_v, rmax_v, facc, out_v,
            sem_x, sem_w, sem_o):
    def x_copy(b):
        rows = pl.ds(pl.multiple_of(b * RB, RB), RB)
        return pltpu.make_async_copy(x_hbm.at[rows], x_v.at[rows], sem_x.at[b])

    w_copies = [pltpu.make_async_copy(src, dst, sem_w.at[i]) for i, (src, dst) in enumerate(
        ((wg_hbm, wg_v), (wu_hbm, wu_v), (wd_hbm, wd_v), (wo_hbm, wo_v)))]

    def out_copy(b):
        rows = pl.ds(pl.multiple_of(b * RB, RB), RB)
        return pltpu.make_async_copy(out_v.at[rows], out_hbm.at[rows], sem_o.at[b])

    wk_copy = pltpu.make_async_copy(wqkv_hbm.at[:, pl.ds(D, D)], wk_v, sem_w.at[5])
    wq_copy = pltpu.make_async_copy(wqkv_hbm.at[:, pl.ds(0, D)], wq_v, sem_w.at[6])
    wv_copy = pltpu.make_async_copy(wqkv_hbm.at[:, pl.ds(2 * D, D)], wv_v, sem_w.at[7])

    def head_indicator():
        hh = lax.broadcasted_iota(jnp.int32, (H, D), 0) * DH
        cc = lax.broadcasted_iota(jnp.int32, (H, D), 1)
        return jnp.where((cc >= hh) & (cc < hh + DH), 1.0, 0.0).astype(bf16)

    x_copy(0).start()
    wk_copy.start()
    kmax_v[...] = jnp.zeros_like(kmax_v)
    rmax_v[...] = jnp.zeros_like(rmax_v)
    x_copy(0).wait()
    for b in range(1, NRB):
        x_copy(b).start()
    wq_copy.start()
    wv_copy.start()
    wk_copy.wait()

    def ln_kproj(b):
        ind = head_indicator()
        kmx = kmax_v[...]
        for i in range(RB // SB):
            r0 = b * RB + i * SB
            rows = pl.ds(r0 if isinstance(b, int) else pl.multiple_of(r0, SB), SB)
            h0 = b * (RB // 2) + i * (SB // 2)
            hrows = pl.ds(h0 if isinstance(b, int) else pl.multiple_of(h0, SB // 2), SB // 2)
            x = x_v[rows, :].astype(f32)
            mu = jnp.mean(x, axis=-1, keepdims=True)
            xc = x - mu
            var = jnp.mean(xc * xc, axis=-1, keepdims=True)
            xn = (xc * lax.rsqrt(var + EPS)).astype(bf16)
            xn_v[rows, :] = xn
            kk = jnp.dot(xn, wk_v[...], preferred_element_type=f32)
            for j in range(5):
                kn_v[j, hrows, :] = pltpu.bitcast(kk[:, j * 128:(j + 1) * 128].astype(bf16), u32)
            n2 = lax.dot_general(ind, (kk * kk).astype(bf16), (((1,), (1,)), ((), ())),
                                 preferred_element_type=f32)
            for t in range(SB // 128):
                kmx = jnp.maximum(kmx, n2[:, t * 128:(t + 1) * 128])
        kmax_v[...] = kmx

    def p1a_body(b, carry):
        ln_kproj(b)
        x_copy(b + 1).wait()
        return carry

    with jax.named_scope("ph1a"):
        lax.fori_loop(0, NRB - 1, p1a_body, 0)

    with jax.named_scope("ph1t"):
        wq_copy.wait()
        wv_copy.wait()
        for c in w_copies:
            c.start()
        ln_kproj(NRB - 1)
        wqvt_v[0:D, :] = wq_v[...].T
        wqvt_v[D:2 * D, :] = wv_v[...].T
        kn = jnp.sqrt(jnp.maximum(jnp.max(kmax_v[...], axis=1, keepdims=True), 1e-30))
        kmax_v[...] = jnp.broadcast_to(kn * MARGIN, (H, 128))

    def p1b_body(b, carry):
        rows = pl.ds(pl.multiple_of(b * RB, RB), RB)
        hrows = pl.ds(pl.multiple_of(b * (RB // 2), RB // 2), RB // 2)
        xn = xn_v[rows, :]
        qt = lax.dot_general(wqvt_v[0:D, :], xn, (((1,), (1,)), ((), ())), preferred_element_type=f32)
        qt = qt * QSCALE
        n2 = jnp.dot(head_indicator(), (qt * qt).astype(bf16), preferred_element_type=f32)
        bound = jnp.sqrt(jnp.maximum(n2, 1e-30)) * jnp.concatenate([kmax_v[...]] * (RB // 128), axis=1)
        rmx = rmax_v[...]
        for t in range(RB // 128):
            bt = bound[:, t * 128:(t + 1) * 128]
            rmx = jnp.where(bt <= rmx, rmx, bt)
        rmax_v[...] = rmx
        inv_eps = bound * (2.0 / G)
        eps = 1.0 / inv_eps
        r8 = lax.broadcasted_iota(jnp.int32, (8, RB), 0)
        crow = jnp.where(r8 == 0, C, 0.0).astype(f32)
        for p in range(NP):
            c0 = 2 * DH * p
            e = eps[2 * p + 1:2 * p + 2, :]
            mid = qt[c0 + 16:c0 + 24, :]
            w = jnp.concatenate([
                qt[c0:c0 + 16, :], jnp.where(r8 < 4, mid, 0.0), crow, -crow,
                jnp.where(r8 >= 4, mid * e, 0.0), qt[c0 + 24:c0 + 40, :] * e], axis=0)
            qm_v[p, :, rows] = pltpu.bitcast(w.astype(bf16), u32)
            ie_v[p, :, rows] = jnp.broadcast_to(inv_eps[2 * p + 1:2 * p + 2, :], (8, RB))
        vt = lax.dot_general(wqvt_v[D:2 * D, :], xn, (((1,), (1,)), ((), ())), preferred_element_type=f32)
        tail = jnp.where(lax.broadcasted_iota(jnp.int32, (R - DH, RB), 0) == 0, 1.0, 0.0).astype(f32)
        for h in range(H):
            vt_v[h, 0:DH, rows] = vt[h * DH:(h + 1) * DH, :]
            vt_v[h, DH:R, rows] = tail
        lane = lax.broadcasted_iota(jnp.int32, (RB // 2, 128), 1)
        for p in range(NP):
            j, o = (2 * DH * p) // 128, (2 * DH * p) % 128
            src = kn_v[j, hrows, :]
            if o + 2 * DH > 128:
                src = jnp.where(lane >= o, src, kn_v[j + 1, hrows, :])
            r1 = src if o == 0 else pltpu.roll(src, 128 - o, 1)
            sh2 = (24 - o) % 128
            r2 = src if sh2 == 0 else pltpu.roll(src, sh2, 1)
            kp_v[p, hrows, :] = jnp.where(lane < 24, r1, jnp.where(lane < 40, jnp.uint32(ONES2), r2))
        return carry

    with jax.named_scope("ph1b"):
        lax.fori_loop(0, NRB, p1b_body, 0)

    def probe_terms(n):
        pc = lax.broadcasted_iota(jnp.int32, (n, 128), 1)
        return (((pc % 64) - 32).astype(f32) * (G / 16),
                ((pc % 7) - 3).astype(f32) * (G / 64))

    pr = lax.broadcasted_iota(jnp.int32, (KR, 128), 0)
    a1, a2 = probe_terms(KR)
    pw = jnp.where(pr == 3, a1, jnp.where(pr == 17, 1.0, jnp.where(pr == 24, C, jnp.where(
        pr == 32, -C, jnp.where((pr == 45) | (pr == 60), a2, 0.0)))))
    pout = jnp.dot(jnp.ones((16, KR), bf16), pw.astype(bf16), preferred_element_type=f32)
    a1, a2 = probe_terms(16)
    pexp = (((a1 + 1.0) + C) - C) + 2.0 * a2
    probe_bad = jnp.max(jnp.where(pout == pexp, 0.0, 1.0))
    range_bad = jnp.max(jnp.where(rmax_v[...] <= RLIM, 0.0, 1.0))
    fast = (probe_bad + range_bad) == 0.0

    for c in w_copies:
        c.wait()

    def silu_mul(g, u):
        hg = 0.5 * g
        return ((hg + hg * jnp.tanh(hg)) * u).astype(bf16)

    def kchunk(p, r0, n):
        return pltpu.bitcast(kp_v[p, r0 // 2:(r0 + n) // 2, :], bf16)[:, 0:KR]

    s1buf, s2buf, m1buf, m2buf = (s1a, s1b), (s2a, s2b), (m1a, m1b), (m2a, m2b)

    def qk_chunk(unit, c, slot, m):
        p, qb = unit
        cols = slice(qb * TQ, (qb + 1) * TQ)
        out = jnp.dot(kchunk(p, c * KC, KC), pltpu.bitcast(qm_v[p, :, cols], bf16),
                      preferred_element_type=f32)
        t = (out + C) - C
        s2 = ((out - t).reshape(KC // 8, 8, TQ) * ie_v[p, :, cols][None])
        s1buf[slot][c * KC:(c + 1) * KC, :] = t
        s2buf[slot][c * KC:(c + 1) * KC, :] = s2.reshape(KC, TQ)
        a = jnp.max(t.reshape(KC // 8, 8, TQ), axis=0)
        b = jnp.max(s2, axis=0)
        return (a, b) if m is None else (jnp.maximum(m[0], a), jnp.maximum(m[1], b))

    def pv_chunk(p, c, slot, m, o):
        rows = slice(c * KC, (c + 1) * KC)
        p1 = jnp.exp2(s1buf[slot][rows, :].reshape(KC // 8, 8, TQ) - m[0][None]).reshape(KC, TQ).astype(PDT)
        p2 = jnp.exp2(s2buf[slot][rows, :].reshape(KC // 8, 8, TQ) - m[1][None]).reshape(KC, TQ).astype(PDT)
        o1 = jnp.dot(vt_v[2 * p, :, rows], p1, preferred_element_type=f32)
        o2 = jnp.dot(vt_v[2 * p + 1, :, rows], p2, preferred_element_type=f32)
        return (o1, o2) if o is None else (o[0] + o1, o[1] + o2)

    def fin(mn, slot):
        m1buf[slot][...] = jnp.broadcast_to(jnp.max(mn[0], axis=0, keepdims=True), (8, TQ))
        m2buf[slot][...] = jnp.broadcast_to(jnp.max(mn[1], axis=0, keepdims=True), (8, TQ))

    def pair_step(p, last):
        pn = p + 1

        def unit(k):
            return (p, k) if k < NQ else (pn, k - NQ)

        frows = pl.ds(p * FR if isinstance(p, int) else pl.multiple_of(p * FR, FR), FR)
        st = {"g": None, "hm": []}

        def tg(i):
            def run():
                st["g"] = jnp.dot(xn_v[frows, :], wg_v[:, i * 128:(i + 1) * 128], preferred_element_type=f32)
            return run

        def tu(i):
            def run():
                uu = jnp.dot(xn_v[frows, :], wu_v[:, i * 128:(i + 1) * 128], preferred_element_type=f32)
                st["hm"].append(silu_mul(st["g"], uu))
            return run

        def td(n):
            def run():
                hmid = jnp.concatenate(st["hm"], axis=1)
                facc[frows, n * 128:(n + 1) * 128] = jnp.dot(
                    hmid, wd_v[:, n * 128:(n + 1) * 128], preferred_element_type=f32)
            return run

        tasks = []
        for i in range(F // 128):
            tasks += [(5, tg(i)), (5, tu(i))]
        tasks += [(F // 128, td(n)) for n in range(D // 128)]
        tot = sum(w for w, _ in tasks)
        done = 0
        cnt = 0
        mn = (mp1[...], mp2[...])
        for u in range(NQ):
            m = (m1buf[u % 2][...], m2buf[u % 2][...])
            o = None
            mn2 = None
            for c in range(NC):
                while tasks and (done + tasks[0][0] / 2) / tot <= (cnt + 0.5) / (NQ * NC - 1):
                    w, run = tasks.pop(0)
                    run()
                    done += w
                cnt += 1
                if c + LAG < NC:
                    if not (last and u + 1 >= NQ):
                        mn = qk_chunk(unit(u + 1), c + LAG, (u + 1) % 2, mn)
                        if c + LAG == NC - 1:
                            fin(mn, (u + 1) % 2)
                    o = pv_chunk(p, c, u % 2, m, o)
                else:
                    o = pv_chunk(p, c, u % 2, m, o)
                    if not (last and u + 2 >= NQ):
                        mn2 = qk_chunk(unit(u + 2), c + LAG - NC, u % 2, mn2)
            for i in range(2):
                ot_v[2 * p + i, :, u * TQ:(u + 1) * TQ] = o[i] * (1.0 / o[i][DH:DH + 1, :])
            mn = mn2
        for w, run in tasks:
            run()
        if not last:
            mp1[...] = mn[0]
            mp2[...] = mn[1]

    @pl.when(fast)
    def _():
        mn = None
        for c in range(NC):
            mn = qk_chunk((0, 0), c, 0, mn)
        fin(mn, 0)
        mn = None
        for c in range(LAG):
            mn = qk_chunk((0, 1), c, 1, mn)
        mp1[...] = mn[0]
        mp2[...] = mn[1]

        def body(p, carry):
            pair_step(p, False)
            return carry

        with jax.named_scope("ph2"):
            lax.fori_loop(0, NP - 1, body, 0)
            pair_step(NP - 1, True)

    @pl.when(jnp.logical_not(fast))
    def _():
        def att_body(i, carry):
            p = i // NQ
            cols = pl.ds(pl.multiple_of((i % NQ) * TQ, TQ), TQ)
            w = pltpu.bitcast(qm_v[p, :, cols], bf16)
            wr = lax.broadcasted_iota(jnp.int32, (KR, TQ), 0)
            kk = kchunk(p, 0, S)
            for k in range(2):
                wk = jnp.where((wr < 24) if k == 0 else (wr >= 40), w, jnp.zeros_like(w))
                s = jnp.dot(kk, wk, preferred_element_type=f32)
                if k == 1:
                    s = s * ie_v[p, 0:1, cols]
                pp = jnp.exp2(s - jnp.max(s, axis=0, keepdims=True)).astype(bf16)
                o = jnp.dot(vt_v[2 * p + k], pp, preferred_element_type=f32)
                ot_v[2 * p + k, :, cols] = o * (1.0 / o[DH:DH + 1, :])
            return carry

        lax.fori_loop(0, NP * NQ, att_body, 0)

        def ffn_body(i, carry):
            rows = pl.ds(pl.multiple_of(i * FR, FR), FR)
            xr = xn_v[rows, :]
            g = jnp.dot(xr, wg_v[...], preferred_element_type=f32)
            uu = jnp.dot(xr, wu_v[...], preferred_element_type=f32)
            facc[rows, :] = jnp.dot(silu_mul(g, uu), wd_v[...], preferred_element_type=f32)
            return carry

        lax.fori_loop(0, NP, ffn_body, 0)

    def p3_body(b, carry):
        rows = pl.ds(pl.multiple_of(b * RB, RB), RB)
        ot = jnp.concatenate([ot_v[h, 0:DH, rows] for h in range(H)], axis=0).astype(bf16)
        attn = lax.dot_general(ot, wo_v[...], (((0,), (0,)), ((), ())), preferred_element_type=f32)
        out_v[rows, :] = (x_v[rows, :].astype(f32) + facc[rows, :] + attn).astype(bf16)
        out_copy(b).start()
        return carry

    with jax.named_scope("ph3"):
        lax.fori_loop(0, NRB, p3_body, 0)
    for b in range(NRB):
        out_copy(b).wait()


PDT = bf16


@jax.jit
def pallas_parallel_sum__mha_block__swiglu_ffn__prompt_kernel(
    A_x: jax.Array,
    A_wqkv: jax.Array,
    A_wo: jax.Array,
    B_x: jax.Array,
    B_w_gate: jax.Array,
    B_w_up: jax.Array,
    B_w_down: jax.Array,
):
    x = A_x.reshape(S, D)
    any_spec = pl.BlockSpec(memory_space=pl.ANY)
    out = pl.pallas_call(
        _kernel,
        out_shape=jax.ShapeDtypeStruct((S, D), bf16),
        in_specs=[any_spec] * 6,
        out_specs=any_spec,
        scratch_shapes=[
            pltpu.VMEM((S, D), bf16),
            pltpu.VMEM((D, D), bf16),
            pltpu.VMEM((D, D), bf16),
            pltpu.VMEM((D, D), bf16),
            pltpu.VMEM((D, D), bf16),
            pltpu.VMEM((D, F), bf16),
            pltpu.VMEM((D, F), bf16),
            pltpu.VMEM((F, D), bf16),
            pltpu.VMEM((2 * D, D), bf16),
            pltpu.VMEM((S, D), bf16),
            pltpu.VMEM((5, S // 2, 128), u32),
            pltpu.VMEM((NP, S // 2, 128), u32),
            pltpu.VMEM((NP, KR // 2, S), u32),
            pltpu.VMEM((NP, 8, S), f32),
            pltpu.VMEM((H, R, S), f32),
            pltpu.VMEM((H, R, S), f32),
        ] + [pltpu.VMEM((S, TQ), f32)] * 4 + [pltpu.VMEM((8, TQ), f32)] * 6 + [
            pltpu.VMEM((H, 128), f32),
            pltpu.VMEM((H, 128), f32),
            pltpu.VMEM((S, D), f32),
            pltpu.VMEM((S, D), bf16),
            pltpu.SemaphoreType.DMA((NRB,)),
            pltpu.SemaphoreType.DMA((8,)),
            pltpu.SemaphoreType.DMA((NRB,)),
        ],
        compiler_params=pltpu.CompilerParams(vmem_limit_bytes=100 * 2**20),
    )(x, A_wqkv, A_wo, B_w_gate, B_w_up, B_w_down)
    return out.reshape(1, S, D)
```

```python
import math

import jax
import jax.numpy as jnp
from jax import lax
import jax.experimental.pallas as pl
import jax.experimental.pallas.tpu as pltpu

S = 2048
D = 640
H = 32
DH = 20
NP = H // 2
F = 1536
R = 24
TQ = 256
KC = 128
LAG = 3
NQ = S // TQ
NC = S // KC
RB = 512
NRB = S // RB
SUBS = (128, 128, 256)
FR = S // NP
EPS = 1e-5
QSCALE = (DH ** -0.5) * math.log2(math.e)

KR = 64
G = 2.0 ** -6
C = 1.5 * 2.0 ** 23 * G
RLIM = 160.0
MARGIN = 1.03
YLIM = (RLIM * 2.0 / G) ** 2
ONES2 = 0x3F803F80

f32 = jnp.float32
bf16 = jnp.bfloat16
u32 = jnp.uint32
i32 = jnp.int32


def _ds(start, size, align):
    return pl.ds(start if isinstance(start, int) else pl.multiple_of(start, align), size)


def _kernel(x_hbm, wqkv_hbm, wo_hbm, wg_hbm, wu_hbm, wd_hbm, out_hbm,
            x_v, wq_v, wk_v, wv_v, wo_v, wg_v, wu_v, wd_v,
            wqvt_v, xn_v, kn_v, kp_v, qm_v, ie_v, vt_v, ot_v,
            s1a, s1b, s2a, s2b, m1a, m1b, m2a, m2b, mp1, mp2,
            kmax_v, bad_v, facc, out_v,
            sem_x, sem_w, sem_o):
    def x_copy(b):
        rows = _ds(b * RB, RB, RB)
        return pltpu.make_async_copy(x_hbm.at[rows], x_v.at[rows], sem_x.at[b])

    def out_copy(b):
        rows = _ds(b * TQ, TQ, TQ)
        return pltpu.make_async_copy(out_v.at[rows], out_hbm.at[rows], sem_o.at[b])

    w_copies = [pltpu.make_async_copy(src, dst, sem_w.at[i]) for i, (src, dst) in enumerate(
        ((wg_hbm, wg_v), (wu_hbm, wu_v), (wd_hbm, wd_v), (wo_hbm, wo_v)))]
    wq_copy = pltpu.make_async_copy(wqkv_hbm.at[:, pl.ds(0, D)], wq_v, sem_w.at[4])
    wk_copy = pltpu.make_async_copy(wqkv_hbm.at[:, pl.ds(D, D)], wk_v, sem_w.at[5])
    wv_copy = pltpu.make_async_copy(wqkv_hbm.at[:, pl.ds(2 * D, D)], wv_v, sem_w.at[6])

    x_copy(0).start()
    wk_copy.start()
    kmax_v[...] = jnp.zeros_like(kmax_v)

    def probe_terms(n):
        pc = lax.broadcasted_iota(i32, (n, 128), 1)
        i1 = 2 * (pc % 64) - 63
        on_grid = lax.shift_right_arithmetic(i1 + 16, 5).astype(f32) * G
        return i1.astype(f32) * (G / 32), on_grid, ((pc % 7) - 3).astype(f32) * (G / 64)

    pr = lax.broadcasted_iota(i32, (KR, 128), 0)
    a1, _, a2 = probe_terms(KR)
    pw = jnp.where(pr == 3, a1, jnp.where(pr == 17, 1.0, jnp.where(pr == 24, C, jnp.where(
        pr == 32, -C, jnp.where((pr == 45) | (pr == 60), a2, 0.0)))))
    pout = jnp.dot(jnp.ones((16, KR), bf16), pw.astype(bf16), preferred_element_type=f32)
    _, a1g, a2 = probe_terms(16)
    pt = (pout + C) - C
    pbad = jnp.where((pt == a1g + 1.0) & (pout - pt == 2.0 * a2), 0.0, 1.0)
    bad_v[...] = jnp.maximum(pbad[0:8], pbad[8:16])

    def layernorm(r0, n):
        x = x_v[_ds(r0, n, 64), :].astype(f32)
        mu = jnp.mean(x, axis=-1, keepdims=True)
        xc = x - mu
        var = jnp.mean(xc * xc, axis=-1, keepdims=True)
        xn = (xc * lax.rsqrt(var + EPS)).astype(bf16)
        xn_v[_ds(r0 // 2, n // 2, 32), :] = pltpu.bitcast(xn, u32)
        return xn

    def xn_rows(r0, n):
        return pltpu.bitcast(xn_v[_ds(r0 // 2, n // 2, 32), :], bf16)

    def kproj(xn, r0, n):
        kk = jnp.dot(xn, wk_v[...], preferred_element_type=f32)
        for j in range(D // 128):
            kn_v[j, _ds(r0 // 2, n // 2, 32), :] = pltpu.bitcast(
                kk[:, j * 128:(j + 1) * 128].astype(bf16), u32)

    def ln_kproj(b):
        off = 0
        for n in SUBS:
            r0 = b * RB + off
            kproj(layernorm(r0, n), r0, n)
            off += n

    def knorm(b):
        hrows = _ds(b * (RB // 2), RB // 2, RB // 2)
        kk = jnp.concatenate([pltpu.bitcast(kn_v[j, hrows, :], bf16) for j in range(D // 128)],
                             axis=1).astype(f32)
        hh = lax.broadcasted_iota(i32, (H, D), 0) * DH
        cc = lax.broadcasted_iota(i32, (H, D), 1)
        ind = jnp.where((cc >= hh) & (cc < hh + DH), 1.0, 0.0).astype(bf16)
        n2 = lax.dot_general(ind, (kk * kk).astype(bf16), (((1,), (1,)), ((), ())),
                             preferred_element_type=f32)
        kmx = kmax_v[...]
        for t in range(RB // 128):
            kmx = jnp.maximum(kmx, n2[:, t * 128:(t + 1) * 128])
        kmax_v[...] = kmx

    def p1a_body(b, carry):
        x_copy(b).wait()
        knorm(b - 1)
        ln_kproj(b)
        return carry

    x_copy(0).wait()
    for b in range(1, NRB):
        x_copy(b).start()
    wq_copy.start()
    wv_copy.start()
    layernorm(0, RB)
    wk_copy.wait()
    kproj(xn_rows(0, RB), 0, RB)
    lax.fori_loop(1, NRB - 1, p1a_body, 0)

    x_copy(NRB - 1).wait()
    wq_copy.wait()
    wv_copy.wait()
    for c in w_copies:
        c.start()
    knorm(NRB - 2)
    ln_kproj(NRB - 1)
    knorm(NRB - 1)
    wqvt_v[0:D, :] = wq_v[...].T
    wqvt_v[D:2 * D, :] = wv_v[...].T
    kn = jnp.maximum(jnp.max(kmax_v[...], axis=1, keepdims=True), 1e-30)
    kmax_v[...] = jnp.broadcast_to(kn * (MARGIN * 2.0 / G) ** 2, (H, 128))

    def p1b_body(b, carry):
        rows = _ds(b * RB, RB, RB)
        hrows = _ds(b * (RB // 2), RB // 2, RB // 2)
        xn = xn_rows(b * RB, RB)
        qt = lax.dot_general(wqvt_v[0:D, :], xn, (((1,), (1,)), ((), ())), preferred_element_type=f32)
        qt = qt * QSCALE
        r8 = lax.broadcasted_iota(i32, (8, RB), 0)
        crow = jnp.where(r8 == 0, C, 0.0).astype(f32)

        def bound2(t0, t1, t2, h):
            n2 = t0 * t0 + t1 * t1 + t2 * t2
            for sh in (4, 2, 1):
                n2 = n2 + pltpu.roll(n2, sh, 0)
            ks = jnp.broadcast_to(kmax_v[h:h + 1, :], (8, 128))
            return jnp.maximum(n2, 1e-30) * jnp.concatenate([ks] * (RB // 128), axis=1)

        bad = jnp.zeros((8, RB), f32)
        for p in range(NP):
            c0 = 2 * DH * p
            a0, a1, mid, b0, b1 = (qt[c0 + 8 * i:c0 + 8 * (i + 1), :] for i in range(5))
            lo = jnp.where(r8 < 4, mid, 0.0)
            hi = jnp.where(r8 >= 4, mid, 0.0)
            y1 = bound2(a0, a1, lo, 2 * p)
            y2 = bound2(hi, b0, b1, 2 * p + 1)
            bad = jnp.where((y1 <= YLIM) & (y2 <= YLIM), bad, 1.0)
            e = lax.shift_right_logical(lax.shift_right_logical(pltpu.bitcast(y2, i32), 23) + 129, 1)
            inv_eps = pltpu.bitcast(lax.shift_left(e, 23), f32)
            eps = pltpu.bitcast(lax.shift_left(254 - e, 23), f32)
            w = jnp.concatenate([a0, a1, lo, crow, -crow, hi * eps, b0 * eps, b1 * eps], axis=0)
            qm_v[p, :, rows] = pltpu.bitcast(w.astype(bf16), u32)
            ie_v[p, :, rows] = inv_eps
        bmx = bad_v[...]
        for t in range(RB // 128):
            bmx = jnp.maximum(bmx, bad[:, t * 128:(t + 1) * 128])
        bad_v[...] = bmx

        vt = lax.dot_general(wqvt_v[D:2 * D, :], xn, (((1,), (1,)), ((), ())), preferred_element_type=f32)
        tail = jnp.where(lax.broadcasted_iota(i32, (R - DH, RB), 0) == 0, 1.0, 0.0).astype(f32)
        for h in range(H):
            vt_v[h, 0:DH, rows] = vt[h * DH:(h + 1) * DH, :]
            vt_v[h, DH:R, rows] = tail

        lane = lax.broadcasted_iota(i32, (RB // 2, 128), 1)
        for p in range(NP):
            j, o = (2 * DH * p) // 128, (2 * DH * p) % 128
            src = kn_v[j, hrows, :]
            if o + 2 * DH > 128:
                src = jnp.where(lane >= o, src, kn_v[j + 1, hrows, :])
            r1 = src if o == 0 else pltpu.roll(src, 128 - o, 1)
            sh2 = (24 - o) % 128
            r2 = src if sh2 == 0 else pltpu.roll(src, sh2, 1)
            kp_v[p, hrows, :] = jnp.where(lane < 24, r1, jnp.where(lane < 40, jnp.uint32(ONES2), r2))
        return carry

    lax.fori_loop(0, NRB, p1b_body, 0)

    for c in w_copies:
        c.wait()
    fast = jnp.max(bad_v[...]) == 0.0

    def silu_mul(g, u):
        hg = 0.5 * g
        return ((hg + hg * jnp.tanh(hg)) * u).astype(bf16)

    def kchunk(p, r0, n):
        return pltpu.bitcast(kp_v[p, r0 // 2:(r0 + n) // 2, :], bf16)[:, 0:KR]

    def oproj_tasks(b):
        rows = _ds(b * TQ, TQ, TQ)
        st = {}

        def tn(n):
            def run():
                if n == 0:
                    st["o"] = jnp.concatenate([ot_v[h, 0:DH, rows] for h in range(H)],
                                              axis=0).astype(bf16).T
                cols = slice(n * 128, (n + 1) * 128)
                attn = jnp.dot(st["o"], wo_v[:, cols], preferred_element_type=f32)
                out_v[rows, cols] = (x_v[rows, cols].astype(f32) + facc[rows, cols] + attn).astype(bf16)
                if n == D // 128 - 1:
                    out_copy(b).start()
            return run

        return [tn(n) for n in range(D // 128)]

    s1buf, s2buf, m1buf, m2buf = (s1a, s1b), (s2a, s2b), (m1a, m1b), (m2a, m2b)

    def qk_chunk(unit, c, slot, m):
        p, qb = unit
        cols = slice(qb * TQ, (qb + 1) * TQ)
        out = jnp.dot(kchunk(p, c * KC, KC), pltpu.bitcast(qm_v[p, :, cols], bf16),
                      preferred_element_type=f32)
        t = (out + C) - C
        s2 = (out - t).reshape(KC // 8, 8, TQ) * ie_v[p, :, cols][None]
        s1buf[slot][c * KC:(c + 1) * KC, :] = t
        s2buf[slot][c * KC:(c + 1) * KC, :] = s2.reshape(KC, TQ)
        a = jnp.max(t.reshape(KC // 8, 8, TQ), axis=0)
        b = jnp.max(s2, axis=0)
        return (a, b) if m is None else (jnp.maximum(m[0], a), jnp.maximum(m[1], b))

    def pv_chunk(p, c, slot, m, o):
        rows = slice(c * KC, (c + 1) * KC)
        p1 = jnp.exp2(s1buf[slot][rows, :].reshape(KC // 8, 8, TQ) - m[0][None]).reshape(KC, TQ)
        p2 = jnp.exp2(s2buf[slot][rows, :].reshape(KC // 8, 8, TQ) - m[1][None]).reshape(KC, TQ)
        o1 = jnp.dot(vt_v[2 * p, :, rows], p1, preferred_element_type=f32)
        o2 = jnp.dot(vt_v[2 * p + 1, :, rows], p2, preferred_element_type=f32)
        return (o1, o2) if o is None else (o[0] + o1, o[1] + o2)

    def fin(mn, slot):
        m1buf[slot][...] = jnp.broadcast_to(jnp.max(mn[0], axis=0, keepdims=True), (8, TQ))
        m2buf[slot][...] = jnp.broadcast_to(jnp.max(mn[1], axis=0, keepdims=True), (8, TQ))

    def pair_step(p, last):
        def unit(k):
            return (p, k) if k < NQ else (p + 1, k - NQ)

        frows = _ds(p * FR, FR, FR)
        st = {"g": None, "hm": []}

        def tg(i):
            def run():
                st["g"] = jnp.dot(xn_rows(p * FR, FR), wg_v[:, i * 128:(i + 1) * 128],
                                  preferred_element_type=f32)
            return run

        def tu(i):
            def run():
                uu = jnp.dot(xn_rows(p * FR, FR), wu_v[:, i * 128:(i + 1) * 128],
                             preferred_element_type=f32)
                st["hm"].append(silu_mul(st["g"], uu))
            return run

        def td(n):
            def run():
                hmid = jnp.concatenate(st["hm"], axis=1)
                facc[frows, n * 128:(n + 1) * 128] = jnp.dot(
                    hmid, wd_v[:, n * 128:(n + 1) * 128], preferred_element_type=f32)
            return run

        tasks = []
        for i in range(F // 128):
            tasks += [(5, tg(i)), (5, tu(i))]
        tasks += [(F // 128, td(n)) for n in range(D // 128)]
        tot = sum(w for w, _ in tasks)
        done = 0
        cnt = 0
        mn = (mp1[...], mp2[...])
        otasks = []
        for u in range(NQ):
            m = (m1buf[u % 2][...], m2buf[u % 2][...])
            o = None
            mn2 = None
            for c in range(NC):
                while tasks and (done + tasks[0][0] / 2) / tot <= (cnt + 0.5) / (NQ * NC - 1):
                    w, run = tasks.pop(0)
                    run()
                    done += w
                cnt += 1
                if otasks and c % 3 == 2:
                    otasks.pop(0)()
                if c + LAG < NC:
                    if not (last and u + 1 >= NQ):
                        mn = qk_chunk(unit(u + 1), c + LAG, (u + 1) % 2, mn)
                        if c + LAG == NC - 1:
                            fin(mn, (u + 1) % 2)
                    o = pv_chunk(p, c, u % 2, m, o)
                else:
                    o = pv_chunk(p, c, u % 2, m, o)
                    if not (last and u + 2 >= NQ):
                        mn2 = qk_chunk(unit(u + 2), c + LAG - NC, u % 2, mn2)
            for i in range(2):
                ot_v[2 * p + i, :, u * TQ:(u + 1) * TQ] = o[i] * (1.0 / o[i][DH:DH + 1, :])
            mn = mn2
            if last:
                otasks = oproj_tasks(u)
        for w, run in tasks:
            run()
        for run in otasks:
            run()
        if not last:
            mp1[...] = mn[0]
            mp2[...] = mn[1]

    mn = None
    for c in range(NC):
        mn = qk_chunk((0, 0), c, 0, mn)
    fin(mn, 0)
    mn = None
    for c in range(LAG):
        mn = qk_chunk((0, 1), c, 1, mn)
    mp1[...] = mn[0]
    mp2[...] = mn[1]

    @pl.when(fast)
    def _():
        def body(p, carry):
            pair_step(p, False)
            return carry

        lax.fori_loop(0, NP - 1, body, 0)
        pair_step(NP - 1, True)

    @pl.when(jnp.logical_not(fast))
    def _():
        def att_body(i, carry):
            p = i // NQ
            cols = _ds((i % NQ) * TQ, TQ, TQ)
            w = pltpu.bitcast(qm_v[p, :, cols], bf16)
            wr = lax.broadcasted_iota(i32, (KR, TQ), 0)
            kk = kchunk(p, 0, S)
            for k in range(2):
                wk = jnp.where((wr < 24) if k == 0 else (wr >= 40), w, jnp.zeros_like(w))
                s = jnp.dot(kk, wk, preferred_element_type=f32)
                if k == 1:
                    s = s * ie_v[p, 0:1, cols]
                pp = jnp.exp2(s - jnp.max(s, axis=0, keepdims=True)).astype(bf16)
                o = jnp.dot(vt_v[2 * p + k], pp, preferred_element_type=f32)
                ot_v[2 * p + k, :, cols] = o * (1.0 / o[DH:DH + 1, :])
            return carry

        lax.fori_loop(0, NP * NQ, att_body, 0)

        def ffn_body(i, carry):
            xr = xn_rows(i * FR, FR)
            g = jnp.dot(xr, wg_v[...], preferred_element_type=f32)
            uu = jnp.dot(xr, wu_v[...], preferred_element_type=f32)
            facc[_ds(i * FR, FR, FR), :] = jnp.dot(silu_mul(g, uu), wd_v[...], preferred_element_type=f32)
            return carry

        lax.fori_loop(0, NP, ffn_body, 0)

        def oproj_body(b, carry):
            for run in oproj_tasks(b):
                run()
            return carry

        lax.fori_loop(0, NQ, oproj_body, 0)

    for b in range(NQ):
        out_copy(b).wait()


@jax.jit
def pallas_parallel_sum__mha_block__swiglu_ffn__prompt_kernel(
    A_x: jax.Array,
    A_wqkv: jax.Array,
    A_wo: jax.Array,
    B_x: jax.Array,
    B_w_gate: jax.Array,
    B_w_up: jax.Array,
    B_w_down: jax.Array,
):
    del B_x
    x = A_x.reshape(S, D)
    any_spec = pl.BlockSpec(memory_space=pl.ANY)
    out = pl.pallas_call(
        _kernel,
        out_shape=jax.ShapeDtypeStruct((S, D), bf16),
        in_specs=[any_spec] * 6,
        out_specs=any_spec,
        scratch_shapes=[
            pltpu.VMEM((S, D), bf16),
            pltpu.VMEM((D, D), bf16),
            pltpu.VMEM((D, D), bf16),
            pltpu.VMEM((D, D), bf16),
            pltpu.VMEM((D, D), bf16),
            pltpu.VMEM((D, F), bf16),
            pltpu.VMEM((D, F), bf16),
            pltpu.VMEM((F, D), bf16),
            pltpu.VMEM((2 * D, D), bf16),
            pltpu.VMEM((S // 2, D), u32),
            pltpu.VMEM((5, S // 2, 128), u32),
            pltpu.VMEM((NP, S // 2, 128), u32),
            pltpu.VMEM((NP, KR // 2, S), u32),
            pltpu.VMEM((NP, 8, S), f32),
            pltpu.VMEM((H, R, S), f32),
            pltpu.VMEM((H, R, S), f32),
        ] + [pltpu.VMEM((S, TQ), f32)] * 4 + [pltpu.VMEM((8, TQ), f32)] * 6 + [
            pltpu.VMEM((H, 128), f32),
            pltpu.VMEM((8, 128), f32),
            pltpu.VMEM((S, D), f32),
            pltpu.VMEM((S, D), bf16),
            pltpu.SemaphoreType.DMA((NRB,)),
            pltpu.SemaphoreType.DMA((7,)),
            pltpu.SemaphoreType.DMA((NQ,)),
        ],
        compiler_params=pltpu.CompilerParams(vmem_limit_bytes=100 * 2**20),
    )(x, A_wqkv, A_wo, B_w_gate, B_w_up, B_w_down)
    return out.reshape(1, S, D)
```

```python
import math

import jax
import jax.numpy as jnp
from jax import lax
import jax.experimental.pallas as pl
import jax.experimental.pallas.tpu as pltpu

S = 2048
D = 640
H = 32
DH = 20
NP = H // 2
F = 1536
R = 24
TQ = 256
KC = 128
LAG = 3
NQ = S // TQ
NC = S // KC
RB = 512
NRB = S // RB
SUBS = (128, 128, 256)
FR = S // NP
EPS = 1e-5
QSCALE = (DH ** -0.5) * math.log2(math.e)

KR = 64
G = 2.0 ** -6
C = 1.5 * 2.0 ** 23 * G
RLIM = 250.0
MARGIN = 1.03
YLIM = (RLIM * 2.0 / G) ** 2
ONES2 = 0x3F803F80

f32 = jnp.float32
bf16 = jnp.bfloat16
u32 = jnp.uint32
i32 = jnp.int32


def _ds(start, size, align):
    return pl.ds(start if isinstance(start, int) else pl.multiple_of(start, align), size)


def _kernel(x_hbm, wqkv_hbm, wo_hbm, wg_hbm, wu_hbm, wd_hbm, out_hbm,
            x_v, wq_v, wk_v, wv_v, wo_v, wg_v, wu_v, wd_v,
            wqvt_v, xn_v, kn_v, kp_v, qm_v, ie_v, vt_v, ot_v,
            s1a, s1b, s2a, s2b, m1a, m1b, m2a, m2b, mp1, mp2,
            kmax_v, bad_v, facc, out_v,
            sem_x, sem_w, sem_o):
    def x_copy(b):
        rows = _ds(b * RB, RB, RB)
        return pltpu.make_async_copy(x_hbm.at[rows], x_v.at[rows], sem_x.at[b])

    def out_copy(b):
        rows = _ds(b * TQ, TQ, TQ)
        return pltpu.make_async_copy(out_v.at[rows], out_hbm.at[rows], sem_o.at[b])

    w_copies = [pltpu.make_async_copy(src, dst, sem_w.at[i]) for i, (src, dst) in enumerate(
        ((wg_hbm, wg_v), (wu_hbm, wu_v), (wd_hbm, wd_v), (wo_hbm, wo_v)))]
    wq_copy = pltpu.make_async_copy(wqkv_hbm.at[:, pl.ds(0, D)], wq_v, sem_w.at[4])
    wk_copy = pltpu.make_async_copy(wqkv_hbm.at[:, pl.ds(D, D)], wk_v, sem_w.at[5])
    wv_copy = pltpu.make_async_copy(wqkv_hbm.at[:, pl.ds(2 * D, D)], wv_v, sem_w.at[6])

    x_copy(0).start()
    wk_copy.start()
    kmax_v[...] = jnp.zeros_like(kmax_v)

    def probe_terms(n):
        pc = lax.broadcasted_iota(i32, (n, 128), 1)
        i1 = 2 * (pc % 64) - 63
        on_grid = lax.shift_right_arithmetic(i1 + 16, 5).astype(f32) * G
        return i1.astype(f32) * (G / 32), on_grid, ((pc % 7) - 3).astype(f32) * (G / 64)

    pr = lax.broadcasted_iota(i32, (KR, 128), 0)
    a1, _, a2 = probe_terms(KR)
    pw = jnp.where(pr == 3, a1, jnp.where(pr == 17, 1.0, jnp.where(pr == 24, C, jnp.where(
        pr == 32, -C, jnp.where((pr == 45) | (pr == 60), a2, 0.0)))))
    pout = jnp.dot(jnp.ones((16, KR), bf16), pw.astype(bf16), preferred_element_type=f32)
    _, a1g, a2 = probe_terms(16)
    pt = (pout + C) - C
    pbad = jnp.where((pt == a1g + 1.0) & (pout - pt == 2.0 * a2), 0.0, 1.0)
    bad_v[...] = jnp.maximum(pbad[0:8], pbad[8:16])

    def layernorm(r0, n):
        x = x_v[_ds(r0, n, 64), :].astype(f32)
        mu = jnp.mean(x, axis=-1, keepdims=True)
        xc = x - mu
        var = jnp.mean(xc * xc, axis=-1, keepdims=True)
        xn = (xc * lax.rsqrt(var + EPS)).astype(bf16)
        xn_v[_ds(r0 // 2, n // 2, 32), :] = pltpu.bitcast(xn, u32)
        return xn

    def xn_rows(r0, n):
        return pltpu.bitcast(xn_v[_ds(r0 // 2, n // 2, 32), :], bf16)

    def kproj(xn, r0, n):
        kk = jnp.dot(xn, wk_v[...], preferred_element_type=f32)
        for j in range(D // 128):
            kn_v[j, _ds(r0 // 2, n // 2, 32), :] = pltpu.bitcast(
                kk[:, j * 128:(j + 1) * 128].astype(bf16), u32)

    def ln_kproj(b):
        off = 0
        for n in SUBS:
            r0 = b * RB + off
            kproj(layernorm(r0, n), r0, n)
            off += n

    def knorm(b):
        hrows = _ds(b * (RB // 2), RB // 2, RB // 2)
        kk = jnp.concatenate([pltpu.bitcast(kn_v[j, hrows, :], bf16) for j in range(D // 128)],
                             axis=1).astype(f32)
        hh = lax.broadcasted_iota(i32, (H, D), 0) * DH
        cc = lax.broadcasted_iota(i32, (H, D), 1)
        ind = jnp.where((cc >= hh) & (cc < hh + DH), 1.0, 0.0).astype(bf16)
        n2 = lax.dot_general(ind, (kk * kk).astype(bf16), (((1,), (1,)), ((), ())),
                             preferred_element_type=f32)
        kmx = kmax_v[...]
        for t in range(RB // 128):
            kmx = jnp.maximum(kmx, n2[:, t * 128:(t + 1) * 128])
        kmax_v[...] = kmx

    def p1a_body(b, carry):
        x_copy(b).wait()
        knorm(b - 1)
        ln_kproj(b)
        return carry

    x_copy(0).wait()
    for b in range(1, NRB):
        x_copy(b).start()
    wq_copy.start()
    wv_copy.start()
    layernorm(0, RB)
    wk_copy.wait()
    kproj(xn_rows(0, RB), 0, RB)
    lax.fori_loop(1, NRB - 1, p1a_body, 0)

    x_copy(NRB - 1).wait()
    wq_copy.wait()
    wv_copy.wait()
    for c in w_copies:
        c.start()
    knorm(NRB - 2)
    ln_kproj(NRB - 1)
    knorm(NRB - 1)
    wqvt_v[0:D, :] = wq_v[...].T
    wqvt_v[D:2 * D, :] = wv_v[...].T
    kn = jnp.maximum(jnp.max(kmax_v[...], axis=1, keepdims=True), 1e-30)
    kmax_v[...] = jnp.broadcast_to(kn * (MARGIN * 2.0 / G) ** 2, (H, 128))

    def p1b_body(b, carry):
        rows = _ds(b * RB, RB, RB)
        hrows = _ds(b * (RB // 2), RB // 2, RB // 2)
        xn = xn_rows(b * RB, RB)
        qt = lax.dot_general(wqvt_v[0:D, :], xn, (((1,), (1,)), ((), ())), preferred_element_type=f32)
        qt = qt * QSCALE
        r8 = lax.broadcasted_iota(i32, (8, RB), 0)
        crow = jnp.where(r8 == 0, C, 0.0).astype(f32)

        def bound2(t0, t1, t2, h):
            n2 = t0 * t0 + t1 * t1 + t2 * t2
            for sh in (4, 2, 1):
                n2 = n2 + pltpu.roll(n2, sh, 0)
            ks = jnp.broadcast_to(kmax_v[h:h + 1, :], (8, 128))
            return jnp.maximum(n2, 1e-30) * jnp.concatenate([ks] * (RB // 128), axis=1)

        bad = jnp.zeros((8, RB), f32)
        for p in range(NP):
            c0 = 2 * DH * p
            a0, a1, mid, b0, b1 = (qt[c0 + 8 * i:c0 + 8 * (i + 1), :] for i in range(5))
            lo = jnp.where(r8 < 4, mid, 0.0)
            hi = jnp.where(r8 >= 4, mid, 0.0)
            y1 = bound2(a0, a1, lo, 2 * p)
            y2 = bound2(hi, b0, b1, 2 * p + 1)
            bad = jnp.where((y1 <= YLIM) & (y2 <= YLIM), bad, 1.0)
            e = lax.shift_right_logical(lax.shift_right_logical(pltpu.bitcast(y2, i32), 23) + 129, 1)
            inv_eps = pltpu.bitcast(lax.shift_left(e, 23), f32)
            eps = pltpu.bitcast(lax.shift_left(254 - e, 23), f32)
            w = jnp.concatenate([a0, a1, lo, crow, -crow, hi * eps, b0 * eps, b1 * eps], axis=0)
            qm_v[p, :, rows] = pltpu.bitcast(w.astype(bf16), u32)
            ie_v[p, :, rows] = inv_eps
        bmx = bad_v[...]
        for t in range(RB // 128):
            bmx = jnp.maximum(bmx, bad[:, t * 128:(t + 1) * 128])
        bad_v[...] = bmx

        vt = lax.dot_general(wqvt_v[D:2 * D, :], xn, (((1,), (1,)), ((), ())), preferred_element_type=f32)
        tail = jnp.where(lax.broadcasted_iota(i32, (R - DH, RB), 0) == 0, 1.0, 0.0).astype(f32)
        for h in range(H):
            vt_v[h, 0:DH, rows] = vt[h * DH:(h + 1) * DH, :]
            vt_v[h, DH:R, rows] = tail

        lane = lax.broadcasted_iota(i32, (RB // 2, 128), 1)
        for p in range(NP):
            j, o = (2 * DH * p) // 128, (2 * DH * p) % 128
            src = kn_v[j, hrows, :]
            if o + 2 * DH > 128:
                src = jnp.where(lane >= o, src, kn_v[j + 1, hrows, :])
            r1 = src if o == 0 else pltpu.roll(src, 128 - o, 1)
            sh2 = (24 - o) % 128
            r2 = src if sh2 == 0 else pltpu.roll(src, sh2, 1)
            kp_v[p, hrows, :] = jnp.where(lane < 24, r1, jnp.where(lane < 40, jnp.uint32(ONES2), r2))
        return carry

    lax.fori_loop(0, NRB, p1b_body, 0)

    for c in w_copies:
        c.wait()
    fast = jnp.max(bad_v[...]) == 0.0

    def silu_mul(g, u):
        hg = 0.5 * g
        return ((hg + hg * jnp.tanh(hg)) * u).astype(bf16)

    def kchunk(p, r0, n):
        return pltpu.bitcast(kp_v[p, r0 // 2:(r0 + n) // 2, :], bf16)[:, 0:KR]

    def oproj_tasks(b):
        rows = _ds(b * TQ, TQ, TQ)
        st = {}

        def tn(n):
            def run():
                if n == 0:
                    st["o"] = jnp.concatenate([ot_v[h, 0:DH, rows] for h in range(H)],
                                              axis=0).astype(bf16).T
                cols = slice(n * 128, (n + 1) * 128)
                attn = jnp.dot(st["o"], wo_v[:, cols], preferred_element_type=f32)
                out_v[rows, cols] = (x_v[rows, cols].astype(f32) + facc[rows, cols] + attn).astype(bf16)
                if n == D // 128 - 1:
                    out_copy(b).start()
            return run

        return [tn(n) for n in range(D // 128)]

    s1buf, s2buf, m1buf, m2buf = (s1a, s1b), (s2a, s2b), (m1a, m1b), (m2a, m2b)

    def qk_chunk(unit, c, slot, m):
        p, qb = unit
        cols = slice(qb * TQ, (qb + 1) * TQ)
        out = jnp.dot(kchunk(p, c * KC, KC), pltpu.bitcast(qm_v[p, :, cols], bf16),
                      preferred_element_type=f32)
        t = (out + C) - C
        s2 = (out - t).reshape(KC // 8, 8, TQ) * ie_v[p, :, cols][None]
        s1buf[slot][c * KC:(c + 1) * KC, :] = t
        s2buf[slot][c * KC:(c + 1) * KC, :] = s2.reshape(KC, TQ)
        a = jnp.max(t.reshape(KC // 8, 8, TQ), axis=0)
        b = jnp.max(s2, axis=0)
        return (a, b) if m is None else (jnp.maximum(m[0], a), jnp.maximum(m[1], b))

    def pv_chunk(p, c, slot, m, o):
        rows = slice(c * KC, (c + 1) * KC)
        p1 = jnp.exp2(s1buf[slot][rows, :].reshape(KC // 8, 8, TQ) - m[0][None]).reshape(KC, TQ)
        p2 = jnp.exp2(s2buf[slot][rows, :].reshape(KC // 8, 8, TQ) - m[1][None]).reshape(KC, TQ)
        o1 = jnp.dot(vt_v[2 * p, :, rows], p1, preferred_element_type=f32)
        o2 = jnp.dot(vt_v[2 * p + 1, :, rows], p2, preferred_element_type=f32)
        return (o1, o2) if o is None else (o[0] + o1, o[1] + o2)

    def fin(mn, slot):
        m1buf[slot][...] = jnp.broadcast_to(jnp.max(mn[0], axis=0, keepdims=True), (8, TQ))
        m2buf[slot][...] = jnp.broadcast_to(jnp.max(mn[1], axis=0, keepdims=True), (8, TQ))

    def pair_step(p, last):
        def unit(k):
            return (p, k) if k < NQ else (p + 1, k - NQ)

        frows = _ds(p * FR, FR, FR)
        st = {"g": None, "hm": []}

        def tg(i):
            def run():
                st["g"] = jnp.dot(xn_rows(p * FR, FR), wg_v[:, i * 128:(i + 1) * 128],
                                  preferred_element_type=f32)
            return run

        def tu(i):
            def run():
                uu = jnp.dot(xn_rows(p * FR, FR), wu_v[:, i * 128:(i + 1) * 128],
                             preferred_element_type=f32)
                st["hm"].append(silu_mul(st["g"], uu))
            return run

        def td(n):
            def run():
                hmid = jnp.concatenate(st["hm"], axis=1)
                facc[frows, n * 128:(n + 1) * 128] = jnp.dot(
                    hmid, wd_v[:, n * 128:(n + 1) * 128], preferred_element_type=f32)
            return run

        tasks = []
        for i in range(F // 128):
            tasks += [(5, tg(i)), (5, tu(i))]
        tasks += [(F // 128, td(n)) for n in range(D // 128)]
        tot = sum(w for w, _ in tasks)
        done = 0
        cnt = 0
        mn = (mp1[...], mp2[...])
        otasks = []
        for u in range(NQ):
            m = (m1buf[u % 2][...], m2buf[u % 2][...])
            o = None
            mn2 = None
            for c in range(NC):
                while tasks and (done + tasks[0][0] / 2) / tot <= (cnt + 0.5) / (NQ * NC - 1):
                    w, run = tasks.pop(0)
                    run()
                    done += w
                cnt += 1
                if otasks and c % 3 == 2:
                    otasks.pop(0)()
                if c + LAG < NC:
                    if not (last and u + 1 >= NQ):
                        mn = qk_chunk(unit(u + 1), c + LAG, (u + 1) % 2, mn)
                        if c + LAG == NC - 1:
                            fin(mn, (u + 1) % 2)
                    o = pv_chunk(p, c, u % 2, m, o)
                else:
                    o = pv_chunk(p, c, u % 2, m, o)
                    if not (last and u + 2 >= NQ):
                        mn2 = qk_chunk(unit(u + 2), c + LAG - NC, u % 2, mn2)
            for i in range(2):
                ot_v[2 * p + i, :, u * TQ:(u + 1) * TQ] = o[i] * (1.0 / o[i][DH:DH + 1, :])
            mn = mn2
            if last:
                otasks = oproj_tasks(u)
        for w, run in tasks:
            run()
        for run in otasks:
            run()
        if not last:
            mp1[...] = mn[0]
            mp2[...] = mn[1]

    mn = None
    for c in range(NC):
        mn = qk_chunk((0, 0), c, 0, mn)
    fin(mn, 0)
    mn = None
    for c in range(LAG):
        mn = qk_chunk((0, 1), c, 1, mn)
    mp1[...] = mn[0]
    mp2[...] = mn[1]

    def packed_path():
        def body(p, carry):
            pair_step(p, False)
            return carry

        lax.fori_loop(0, NP - 1, body, 0)
        pair_step(NP - 1, True)

    def plain_path():
        def att_body(i, carry):
            p = i // NQ
            cols = _ds((i % NQ) * TQ, TQ, TQ)
            w = pltpu.bitcast(qm_v[p, :, cols], bf16)
            wr = lax.broadcasted_iota(i32, (KR, TQ), 0)
            kk = kchunk(p, 0, S)
            for k in range(2):
                wk = jnp.where((wr < 24) if k == 0 else (wr >= 40), w, jnp.zeros_like(w))
                s = jnp.dot(kk, wk, preferred_element_type=f32)
                if k == 1:
                    s = s * ie_v[p, 0:1, cols]
                pp = jnp.exp2(s - jnp.max(s, axis=0, keepdims=True)).astype(bf16)
                o = jnp.dot(vt_v[2 * p + k], pp, preferred_element_type=f32)
                ot_v[2 * p + k, :, cols] = o * (1.0 / o[DH:DH + 1, :])
            return carry

        lax.fori_loop(0, NP * NQ, att_body, 0)

        def ffn_body(i, carry):
            xr = xn_rows(i * FR, FR)
            g = jnp.dot(xr, wg_v[...], preferred_element_type=f32)
            uu = jnp.dot(xr, wu_v[...], preferred_element_type=f32)
            facc[_ds(i * FR, FR, FR), :] = jnp.dot(silu_mul(g, uu), wd_v[...], preferred_element_type=f32)
            return carry

        lax.fori_loop(0, NP, ffn_body, 0)

        def oproj_body(b, carry):
            for run in oproj_tasks(b):
                run()
            return carry

        lax.fori_loop(0, NQ, oproj_body, 0)

    lax.cond(fast, packed_path, plain_path)
    for b in range(NQ):
        out_copy(b).wait()


@jax.jit
def pallas_parallel_sum__mha_block__swiglu_ffn__prompt_kernel(
    A_x: jax.Array,
    A_wqkv: jax.Array,
    A_wo: jax.Array,
    B_x: jax.Array,
    B_w_gate: jax.Array,
    B_w_up: jax.Array,
    B_w_down: jax.Array,
):
    del B_x
    x = A_x.reshape(S, D)
    any_spec = pl.BlockSpec(memory_space=pl.ANY)
    out = pl.pallas_call(
        _kernel,
        out_shape=jax.ShapeDtypeStruct((S, D), bf16),
        in_specs=[any_spec] * 6,
        out_specs=any_spec,
        scratch_shapes=[
            pltpu.VMEM((S, D), bf16),
            pltpu.VMEM((D, D), bf16),
            pltpu.VMEM((D, D), bf16),
            pltpu.VMEM((D, D), bf16),
            pltpu.VMEM((D, D), bf16),
            pltpu.VMEM((D, F), bf16),
            pltpu.VMEM((D, F), bf16),
            pltpu.VMEM((F, D), bf16),
            pltpu.VMEM((2 * D, D), bf16),
            pltpu.VMEM((S // 2, D), u32),
            pltpu.VMEM((5, S // 2, 128), u32),
            pltpu.VMEM((NP, S // 2, 128), u32),
            pltpu.VMEM((NP, KR // 2, S), u32),
            pltpu.VMEM((NP, 8, S), f32),
            pltpu.VMEM((H, R, S), f32),
            pltpu.VMEM((H, R, S), f32),
        ] + [pltpu.VMEM((S, TQ), f32)] * 4 + [pltpu.VMEM((8, TQ), f32)] * 6 + [
            pltpu.VMEM((H, 128), f32),
            pltpu.VMEM((8, 128), f32),
            pltpu.VMEM((S, D), f32),
            pltpu.VMEM((S, D), bf16),
            pltpu.SemaphoreType.DMA((NRB,)),
            pltpu.SemaphoreType.DMA((7,)),
            pltpu.SemaphoreType.DMA((NQ,)),
        ],
        compiler_params=pltpu.CompilerParams(vmem_limit_bytes=100 * 2**20),
    )(x, A_wqkv, A_wo, B_w_gate, B_w_up, B_w_down)
    return out.reshape(1, S, D)
```

```python
import math

import jax
import jax.numpy as jnp
from jax import lax
import jax.experimental.pallas as pl
import jax.experimental.pallas.tpu as pltpu

S = 2048
D = 640
H = 32
DH = 20
NP = H // 2
F = 1536
R = 24
TQ = 256
KC = 128
LAG = 3
NQ = S // TQ
NC = S // KC
RB = 512
NRB = S // RB
SUBS = (128, 128, 256)
FR = S // NP
WKA = 256
EPS = 1e-5
QSCALE = (DH ** -0.5) * math.log2(math.e)

KR = 64
G = 2.0 ** -6
C = 1.5 * 2.0 ** 23 * G
RLIM = 250.0
MARGIN = 1.03
YLIM = (RLIM * 2.0 / G) ** 2
ONES2 = 0x3F803F80

f32 = jnp.float32
bf16 = jnp.bfloat16
u32 = jnp.uint32
i32 = jnp.int32


def _ds(start, size, align):
    return pl.ds(start if isinstance(start, int) else pl.multiple_of(start, align), size)


def _kernel(x_hbm, wqkv_hbm, wo_hbm, wg_hbm, wu_hbm, wd_hbm, out_hbm,
            x_v, wq_v, wk_v, wv_v, wo_v, wg_v, wu_v, wd_v,
            wqvt_v, xn_v, kn_v, kp_v, qm_v, ie_v, vt_v, ot_v,
            s1a, s1b, s2a, s2b, m1a, m1b, m2a, m2b, mp1, mp2,
            kmax_v, bad_v, facc, out_v,
            sem_x, sem_w, sem_o):
    def x_copy(b):
        rows = _ds(b * RB, RB, RB)
        return pltpu.make_async_copy(x_hbm.at[rows], x_v.at[rows], sem_x.at[b])

    def out_copy(b):
        rows = _ds(b * TQ, TQ, TQ)
        return pltpu.make_async_copy(out_v.at[rows], out_hbm.at[rows], sem_o.at[b])

    w_copies = [pltpu.make_async_copy(src, dst, sem_w.at[i]) for i, (src, dst) in enumerate(
        ((wg_hbm, wg_v), (wu_hbm, wu_v), (wd_hbm, wd_v), (wo_hbm, wo_v)))]
    wq_copy = pltpu.make_async_copy(wqkv_hbm.at[:, pl.ds(0, D)], wq_v, sem_w.at[4])
    wka_copy = pltpu.make_async_copy(wqkv_hbm.at[:, pl.ds(D, WKA)], wk_v.at[:, pl.ds(0, WKA)], sem_w.at[5])
    wkb_copy = pltpu.make_async_copy(wqkv_hbm.at[:, pl.ds(D + WKA, D - WKA)],
                                     wk_v.at[:, pl.ds(WKA, D - WKA)], sem_w.at[7])
    wv_copy = pltpu.make_async_copy(wqkv_hbm.at[:, pl.ds(2 * D, D)], wv_v, sem_w.at[6])

    x_copy(0).start()
    wka_copy.start()
    kmax_v[...] = jnp.zeros_like(kmax_v)

    def probe_terms(n):
        pc = lax.broadcasted_iota(i32, (n, 128), 1)
        i1 = 2 * (pc % 64) - 63
        on_grid = lax.shift_right_arithmetic(i1 + 16, 5).astype(f32) * G
        return i1.astype(f32) * (G / 32), on_grid, ((pc % 7) - 3).astype(f32) * (G / 64)

    pr = lax.broadcasted_iota(i32, (KR, 128), 0)
    a1, _, a2 = probe_terms(KR)
    pw = jnp.where(pr == 3, a1, jnp.where(pr == 17, 1.0, jnp.where(pr == 24, C, jnp.where(
        pr == 32, -C, jnp.where((pr == 45) | (pr == 60), a2, 0.0)))))
    pout = jnp.dot(jnp.ones((16, KR), bf16), pw.astype(bf16), preferred_element_type=f32)
    _, a1g, a2 = probe_terms(16)
    pt = (pout + C) - C
    pbad = jnp.where((pt == a1g + 1.0) & (pout - pt == 2.0 * a2), 0.0, 1.0)
    bad_v[...] = jnp.maximum(pbad[0:8], pbad[8:16])

    def layernorm(r0, n):
        x = x_v[_ds(r0, n, 64), :].astype(f32)
        mu = jnp.mean(x, axis=-1, keepdims=True)
        xc = x - mu
        var = jnp.mean(xc * xc, axis=-1, keepdims=True)
        xn = (xc * lax.rsqrt(var + EPS)).astype(bf16)
        xn_v[_ds(r0 // 2, n // 2, 32), :] = pltpu.bitcast(xn, u32)
        return xn

    def xn_rows(r0, n):
        return pltpu.bitcast(xn_v[_ds(r0 // 2, n // 2, 32), :], bf16)

    def kproj(xn, r0, n, c0=0, c1=D):
        kk = jnp.dot(xn, wk_v[:, c0:c1], preferred_element_type=f32)
        for j in range((c1 - c0) // 128):
            kn_v[c0 // 128 + j, _ds(r0 // 2, n // 2, 32), :] = pltpu.bitcast(
                kk[:, j * 128:(j + 1) * 128].astype(bf16), u32)

    def ln_kproj(b):
        off = 0
        for n in SUBS:
            r0 = b * RB + off
            kproj(layernorm(r0, n), r0, n)
            off += n

    def knorm(b):
        hrows = _ds(b * (RB // 2), RB // 2, RB // 2)
        kk = jnp.concatenate([pltpu.bitcast(kn_v[j, hrows, :], bf16) for j in range(D // 128)],
                             axis=1).astype(f32)
        hh = lax.broadcasted_iota(i32, (H, D), 0) * DH
        cc = lax.broadcasted_iota(i32, (H, D), 1)
        ind = jnp.where((cc >= hh) & (cc < hh + DH), 1.0, 0.0).astype(bf16)
        n2 = lax.dot_general(ind, (kk * kk).astype(bf16), (((1,), (1,)), ((), ())),
                             preferred_element_type=f32)
        kmx = kmax_v[...]
        for t in range(RB // 128):
            kmx = jnp.maximum(kmx, n2[:, t * 128:(t + 1) * 128])
        kmax_v[...] = kmx

    def p1a_body(b, carry):
        x_copy(b).wait()
        knorm(b - 1)
        ln_kproj(b)
        return carry

    x_copy(0).wait()
    wkb_copy.start()
    layernorm(0, RB)
    wka_copy.wait()
    x_copy(1).start()
    kproj(xn_rows(0, RB), 0, RB, 0, WKA)
    wkb_copy.wait()
    for b in range(2, NRB):
        x_copy(b).start()
    wq_copy.start()
    wv_copy.start()
    kproj(xn_rows(0, RB), 0, RB, WKA, D)
    lax.fori_loop(1, NRB - 1, p1a_body, 0)

    x_copy(NRB - 1).wait()
    wq_copy.wait()
    wv_copy.wait()
    for c in w_copies:
        c.start()
    knorm(NRB - 2)
    ln_kproj(NRB - 1)
    knorm(NRB - 1)
    wqvt_v[0:D, :] = wq_v[...].T
    wqvt_v[D:2 * D, :] = wv_v[...].T
    kn = jnp.maximum(jnp.max(kmax_v[...], axis=1, keepdims=True), 1e-30)
    kmax_v[...] = jnp.broadcast_to(kn * (MARGIN * 2.0 / G) ** 2, (H, 128))

    def p1b_body(b, carry):
        rows = _ds(b * RB, RB, RB)
        hrows = _ds(b * (RB // 2), RB // 2, RB // 2)
        xn = xn_rows(b * RB, RB)
        qt = lax.dot_general(wqvt_v[0:D, :], xn, (((1,), (1,)), ((), ())), preferred_element_type=f32)
        qt = qt * QSCALE
        r8 = lax.broadcasted_iota(i32, (8, RB), 0)
        crow = jnp.where(r8 == 0, C, 0.0).astype(f32)

        def bound2(t0, t1, t2, h):
            n2 = t0 * t0 + t1 * t1 + t2 * t2
            for sh in (4, 2, 1):
                n2 = n2 + pltpu.roll(n2, sh, 0)
            ks = jnp.broadcast_to(kmax_v[h:h + 1, :], (8, 128))
            return jnp.maximum(n2, 1e-30) * jnp.concatenate([ks] * (RB // 128), axis=1)

        bad = jnp.zeros((8, RB), f32)
        for p in range(NP):
            c0 = 2 * DH * p
            a0, a1, mid, b0, b1 = (qt[c0 + 8 * i:c0 + 8 * (i + 1), :] for i in range(5))
            lo = jnp.where(r8 < 4, mid, 0.0)
            hi = jnp.where(r8 >= 4, mid, 0.0)
            y1 = bound2(a0, a1, lo, 2 * p)
            y2 = bound2(hi, b0, b1, 2 * p + 1)
            bad = jnp.where((y1 <= YLIM) & (y2 <= YLIM), bad, 1.0)
            e = lax.shift_right_logical(lax.shift_right_logical(pltpu.bitcast(y2, i32), 23) + 129, 1)
            inv_eps = pltpu.bitcast(lax.shift_left(e, 23), f32)
            eps = pltpu.bitcast(lax.shift_left(254 - e, 23), f32)
            w = jnp.concatenate([a0, a1, lo, crow, -crow, hi * eps, b0 * eps, b1 * eps], axis=0)
            qm_v[p, :, rows] = pltpu.bitcast(w.astype(bf16), u32)
            ie_v[p, :, rows] = inv_eps
        bmx = bad_v[...]
        for t in range(RB // 128):
            bmx = jnp.maximum(bmx, bad[:, t * 128:(t + 1) * 128])
        bad_v[...] = bmx

        vt = lax.dot_general(wqvt_v[D:2 * D, :], xn, (((1,), (1,)), ((), ())), preferred_element_type=f32)
        tail = jnp.where(lax.broadcasted_iota(i32, (R - DH, RB), 0) == 0, 1.0, 0.0).astype(f32)
        for h in range(H):
            vt_v[h, 0:DH, rows] = vt[h * DH:(h + 1) * DH, :]
            vt_v[h, DH:R, rows] = tail

        lane = lax.broadcasted_iota(i32, (RB // 2, 128), 1)
        for p in range(NP):
            j, o = (2 * DH * p) // 128, (2 * DH * p) % 128
            src = kn_v[j, hrows, :]
            if o + 2 * DH > 128:
                src = jnp.where(lane >= o, src, kn_v[j + 1, hrows, :])
            r1 = src if o == 0 else pltpu.roll(src, 128 - o, 1)
            sh2 = (24 - o) % 128
            r2 = src if sh2 == 0 else pltpu.roll(src, sh2, 1)
            kp_v[p, hrows, :] = jnp.where(lane < 24, r1, jnp.where(lane < 40, jnp.uint32(ONES2), r2))
        return carry

    lax.fori_loop(0, NRB, p1b_body, 0)

    for c in w_copies:
        c.wait()
    fast = jnp.max(bad_v[...]) == 0.0

    def silu_mul(g, u):
        hg = 0.5 * g
        return ((hg + hg * jnp.tanh(hg)) * u).astype(bf16)

    def kchunk(p, r0, n):
        return pltpu.bitcast(kp_v[p, r0 // 2:(r0 + n) // 2, :], bf16)[:, 0:KR]

    def oproj_tasks(b):
        rows = _ds(b * TQ, TQ, TQ)
        st = {}

        def tn(n):
            def run():
                if n == 0:
                    st["o"] = jnp.concatenate([ot_v[h, 0:DH, rows] for h in range(H)],
                                              axis=0).astype(bf16).T
                cols = slice(n * 128, (n + 1) * 128)
                attn = jnp.dot(st["o"], wo_v[:, cols], preferred_element_type=f32)
                out_v[rows, cols] = (x_v[rows, cols].astype(f32) + facc[rows, cols] + attn).astype(bf16)
                if n == D // 128 - 1:
                    out_copy(b).start()
            return run

        return [tn(n) for n in range(D // 128)]

    s1buf, s2buf, m1buf, m2buf = (s1a, s1b), (s2a, s2b), (m1a, m1b), (m2a, m2b)

    def qk_chunk(unit, c, slot, m):
        p, qb = unit
        cols = slice(qb * TQ, (qb + 1) * TQ)
        out = jnp.dot(kchunk(p, c * KC, KC), pltpu.bitcast(qm_v[p, :, cols], bf16),
                      preferred_element_type=f32)
        t = (out + C) - C
        s2 = (out - t).reshape(KC // 8, 8, TQ) * ie_v[p, :, cols][None]
        s1buf[slot][c * KC:(c + 1) * KC, :] = t
        s2buf[slot][c * KC:(c + 1) * KC, :] = s2.reshape(KC, TQ)
        a = jnp.max(t.reshape(KC // 8, 8, TQ), axis=0)
        b = jnp.max(s2, axis=0)
        return (a, b) if m is None else (jnp.maximum(m[0], a), jnp.maximum(m[1], b))

    def pv_chunk(p, c, slot, m, o):
        rows = slice(c * KC, (c + 1) * KC)
        p1 = jnp.exp2(s1buf[slot][rows, :].reshape(KC // 8, 8, TQ) - m[0][None]).reshape(KC, TQ)
        p2 = jnp.exp2(s2buf[slot][rows, :].reshape(KC // 8, 8, TQ) - m[1][None]).reshape(KC, TQ)
        o1 = jnp.dot(vt_v[2 * p, :, rows], p1, preferred_element_type=f32)
        o2 = jnp.dot(vt_v[2 * p + 1, :, rows], p2, preferred_element_type=f32)
        return (o1, o2) if o is None else (o[0] + o1, o[1] + o2)

    def fin(mn, slot):
        m1buf[slot][...] = jnp.broadcast_to(jnp.max(mn[0], axis=0, keepdims=True), (8, TQ))
        m2buf[slot][...] = jnp.broadcast_to(jnp.max(mn[1], axis=0, keepdims=True), (8, TQ))

    def pair_step(p, last):
        def unit(k):
            return (p, k) if k < NQ else (p + 1, k - NQ)

        frows = _ds(p * FR, FR, FR)
        st = {"g": None, "hm": []}

        def tg(i):
            def run():
                st["g"] = jnp.dot(xn_rows(p * FR, FR), wg_v[:, i * 128:(i + 1) * 128],
                                  preferred_element_type=f32)
            return run

        def tu(i):
            def run():
                uu = jnp.dot(xn_rows(p * FR, FR), wu_v[:, i * 128:(i + 1) * 128],
                             preferred_element_type=f32)
                st["hm"].append(silu_mul(st["g"], uu))
            return run

        def td(n):
            def run():
                hmid = jnp.concatenate(st["hm"], axis=1)
                facc[frows, n * 128:(n + 1) * 128] = jnp.dot(
                    hmid, wd_v[:, n * 128:(n + 1) * 128], preferred_element_type=f32)
            return run

        tasks = []
        for i in range(F // 128):
            tasks += [(5, tg(i)), (5, tu(i))]
        tasks += [(F // 128, td(n)) for n in range(D // 128)]
        tot = sum(w for w, _ in tasks)
        done = 0
        cnt = 0
        mn = (mp1[...], mp2[...])
        otasks = []
        for u in range(NQ):
            m = (m1buf[u % 2][...], m2buf[u % 2][...])
            o = None
            mn2 = None
            for c in range(NC):
                while tasks and (done + tasks[0][0] / 2) / tot <= (cnt + 0.5) / (NQ * NC - 1):
                    w, run = tasks.pop(0)
                    run()
                    done += w
                cnt += 1
                if otasks and c % 3 == 2:
                    otasks.pop(0)()
                if c + LAG < NC:
                    if not (last and u + 1 >= NQ):
                        mn = qk_chunk(unit(u + 1), c + LAG, (u + 1) % 2, mn)
                        if c + LAG == NC - 1:
                            fin(mn, (u + 1) % 2)
                    o = pv_chunk(p, c, u % 2, m, o)
                else:
                    o = pv_chunk(p, c, u % 2, m, o)
                    if not (last and u + 2 >= NQ):
                        mn2 = qk_chunk(unit(u + 2), c + LAG - NC, u % 2, mn2)
            for i in range(2):
                ot_v[2 * p + i, :, u * TQ:(u + 1) * TQ] = o[i] * (1.0 / o[i][DH:DH + 1, :])
            mn = mn2
            if last:
                otasks = oproj_tasks(u)
        for w, run in tasks:
            run()
        for run in otasks:
            run()
        if not last:
            mp1[...] = mn[0]
            mp2[...] = mn[1]

    mn = None
    for c in range(NC):
        mn = qk_chunk((0, 0), c, 0, mn)
    fin(mn, 0)
    mn = None
    for c in range(LAG):
        mn = qk_chunk((0, 1), c, 1, mn)
    mp1[...] = mn[0]
    mp2[...] = mn[1]

    def packed_path():
        def body(p, carry):
            pair_step(p, False)
            return carry

        lax.fori_loop(0, NP - 1, body, 0)
        pair_step(NP - 1, True)

    def plain_path():
        def att_body(i, carry):
            p = i // NQ
            cols = _ds((i % NQ) * TQ, TQ, TQ)
            w = pltpu.bitcast(qm_v[p, :, cols], bf16)
            wr = lax.broadcasted_iota(i32, (KR, TQ), 0)
            kk = kchunk(p, 0, S)
            for k in range(2):
                wk = jnp.where((wr < 24) if k == 0 else (wr >= 40), w, jnp.zeros_like(w))
                s = jnp.dot(kk, wk, preferred_element_type=f32)
                if k == 1:
                    s = s * ie_v[p, 0:1, cols]
                pp = jnp.exp2(s - jnp.max(s, axis=0, keepdims=True)).astype(bf16)
                o = jnp.dot(vt_v[2 * p + k], pp, preferred_element_type=f32)
                ot_v[2 * p + k, :, cols] = o * (1.0 / o[DH:DH + 1, :])
            return carry

        lax.fori_loop(0, NP * NQ, att_body, 0)

        def ffn_body(i, carry):
            xr = xn_rows(i * FR, FR)
            g = jnp.dot(xr, wg_v[...], preferred_element_type=f32)
            uu = jnp.dot(xr, wu_v[...], preferred_element_type=f32)
            facc[_ds(i * FR, FR, FR), :] = jnp.dot(silu_mul(g, uu), wd_v[...], preferred_element_type=f32)
            return carry

        lax.fori_loop(0, NP, ffn_body, 0)

        def oproj_body(b, carry):
            for run in oproj_tasks(b):
                run()
            return carry

        lax.fori_loop(0, NQ, oproj_body, 0)

    lax.cond(fast, packed_path, plain_path)
    for b in range(NQ):
        out_copy(b).wait()


@jax.jit
def pallas_parallel_sum__mha_block__swiglu_ffn__prompt_kernel(
    A_x: jax.Array,
    A_wqkv: jax.Array,
    A_wo: jax.Array,
    B_x: jax.Array,
    B_w_gate: jax.Array,
    B_w_up: jax.Array,
    B_w_down: jax.Array,
):
    del B_x
    x = A_x.reshape(S, D)
    any_spec = pl.BlockSpec(memory_space=pl.ANY)
    out = pl.pallas_call(
        _kernel,
        out_shape=jax.ShapeDtypeStruct((S, D), bf16),
        in_specs=[any_spec] * 6,
        out_specs=any_spec,
        scratch_shapes=[
            pltpu.VMEM((S, D), bf16),
            pltpu.VMEM((D, D), bf16),
            pltpu.VMEM((D, D), bf16),
            pltpu.VMEM((D, D), bf16),
            pltpu.VMEM((D, D), bf16),
            pltpu.VMEM((D, F), bf16),
            pltpu.VMEM((D, F), bf16),
            pltpu.VMEM((F, D), bf16),
            pltpu.VMEM((2 * D, D), bf16),
            pltpu.VMEM((S // 2, D), u32),
            pltpu.VMEM((5, S // 2, 128), u32),
            pltpu.VMEM((NP, S // 2, 128), u32),
            pltpu.VMEM((NP, KR // 2, S), u32),
            pltpu.VMEM((NP, 8, S), f32),
            pltpu.VMEM((H, R, S), f32),
            pltpu.VMEM((H, R, S), f32),
        ] + [pltpu.VMEM((S, TQ), f32)] * 4 + [pltpu.VMEM((8, TQ), f32)] * 6 + [
            pltpu.VMEM((H, 128), f32),
            pltpu.VMEM((8, 128), f32),
            pltpu.VMEM((S, D), f32),
            pltpu.VMEM((S, D), bf16),
            pltpu.SemaphoreType.DMA((NRB,)),
            pltpu.SemaphoreType.DMA((8,)),
            pltpu.SemaphoreType.DMA((NQ,)),
        ],
        compiler_params=pltpu.CompilerParams(vmem_limit_bytes=100 * 2**20),
    )(x, A_wqkv, A_wo, B_w_gate, B_w_up, B_w_down)
    return out.reshape(1, S, D)
```
